```python
import jax
import jax.numpy as jnp

def _softmax(x, axis=-1):
    return jax.nn.softmax(x, axis=axis)
def _gelu(x):
    return jax.nn.gelu(x, approximate=True)
def _silu(x):
    return jax.nn.silu(x)
def _sigmoid(x):
    return jax.nn.sigmoid(x)
def _layernorm(x, axis=-1, eps=1e-5):
    m = jnp.mean(x, axis=axis, keepdims=True)
    v = jnp.var(x, axis=axis, keepdims=True)
    return (x - m) / jnp.sqrt(v + eps)
def _scatter_add(tgt, idx, src, axis=0):
    return tgt.at[idx].add(src)
def _segment_sum(src, seg, n):
    return jax.ops.segment_sum(src, seg, n)
class _Rng:
    def __init__(self, key):
        self._k = key
    def _next(self):
        self._k, sub = jax.random.split(self._k)
        return sub
    def normal(self, shape):
        return jax.random.normal(self._next(), shape, dtype=jnp.bfloat16)
    def randint(self, lo, hi, shape):
        return jax.random.randint(self._next(), shape, lo, hi, dtype=jnp.int32)
    def uniform(self, shape, lo=0.0, hi=1.0):
        return jax.random.uniform(self._next(), shape, jnp.bfloat16, lo, hi)
    def permutation(self, n):
        return jax.random.permutation(self._next(), n)


kernel_name = 'gated_mix__compressed_kv_cla__gqa_block_cached__decode'

def setup_inputs():
    _rng = _Rng(jax.random.key(int.from_bytes(__import__("os").urandom(4), "little")))
    _w = (lambda a: (lambda t: t.astype(jnp.bfloat16) if jnp.issubdtype(t.dtype, jnp.floating) else t)(jnp.asarray(a)))
    def _A_setup():
        B, H, Sq, Sk, D, M = 1, 32, 1, 4096, 128, 640
        Dc = 4 * D
        return {
            "x": _w((lambda *s: _rng.normal(s) * 0.05)(B, Sq, M)),
            "c_kv": _w((lambda *s: _rng.normal(s) * 0.05)(B, Sk, Dc)),
            "w_q": _w((lambda *s: _rng.normal(s) * 0.05)(M, H, D) * (M ** -0.5)),
            "w_uk": _w((lambda *s: _rng.normal(s) * 0.05)(Dc, H, D) * (Dc ** -0.5)),
            "w_uv": _w((lambda *s: _rng.normal(s) * 0.05)(Dc, H, D) * (Dc ** -0.5)),
            "w_o": _w((lambda *s: _rng.normal(s) * 0.05)(H, D, M) * ((H * D) ** -0.5)),
        }
    _A_in = _A_setup()

    def _B_setup():
        B, Sq, D = 1, 1, 640
        Hq, Hkv, Sk, Dh = 32, 32, 4096, 128
        assert Hq % Hkv == 0, (Hq, Hkv)
        return {
            "x": _w((lambda *s: _rng.normal(s) * 0.05)(B, Sq, D)),
            "k_cache": _w((lambda *s: _rng.normal(s) * 0.05)(B, Hkv, Sk, Dh)),
            "v_cache": _w((lambda *s: _rng.normal(s) * 0.05)(B, Hkv, Sk, Dh)),
            "wq": _w((lambda *s: _rng.normal(s) * 0.05)(D, Hq * Dh) * (D ** -0.5)),
            "wo": _w((lambda *s: _rng.normal(s) * 0.05)(Hq * Dh, D) * ((Hq * Dh) ** -0.5)),
        }
    _B_in = _B_setup()

    return {
        "A_x": _A_in["x"],
        "A_c_kv": _A_in["c_kv"],
        "A_w_q": _A_in["w_q"],
        "A_w_uk": _A_in["w_uk"],
        "A_w_uv": _A_in["w_uv"],
        "A_w_o": _A_in["w_o"],
        "B_x": _B_in["x"],
        "B_k_cache": _B_in["k_cache"],
        "B_v_cache": _B_in["v_cache"],
        "B_wq": _B_in["wq"],
        "B_wo": _B_in["wo"],
        "gate_w": _w((lambda *s: _rng.normal(s) * 0.05)(640)),
    }

def reference(A_x, A_c_kv, A_w_q, A_w_uk, A_w_uv, A_w_o, B_x, B_k_cache, B_v_cache, B_wq, B_wo, gate_w):
    def _A_ref(x, c_kv, w_q, w_uk, w_uv, w_o):
        B, Sq, M = x.shape[0], x.shape[1], x.shape[2]
        Sk = c_kv.shape[1]
        H, D = w_q.shape[1], w_q.shape[2]
        q = jnp.einsum("bqm,mhd->bhqd", x, w_q)
        k = jnp.einsum("bkc,chd->bhkd", c_kv, w_uk)
        v = jnp.einsum("bkc,chd->bhkd", c_kv, w_uv)
        scores = jnp.einsum("bhqd,bhkd->bhqk", q, k) * (D ** -0.5)
        off = Sk - Sq
        qi = jnp.arange(Sq)[:, None]
        kj = jnp.arange(Sk)[None, :]
        cmask = kj <= (qi + off)
        scores = jnp.where(cmask[None, None], scores, -1e9)
        p = _softmax(scores, axis=-1)
        ctx = jnp.einsum("bhqk,bhkd->bhqd", p, v)
        return jnp.einsum("bhqd,hdm->bqm", ctx, w_o)

    def _B_ref(x, k_cache, v_cache, wq, wo):
        B, Sq, D = x.shape
        Hq, Dh = 32, 128
        Hkv = k_cache.shape[1]
        rep = Hq // Hkv
        q = (lambda x, *d: x.transpose(*d))((x @ wq).reshape(B, Sq, Hq, Dh), 0, 2, 1, 3)
        k = jnp.repeat(k_cache, rep, axis=1)
        v = jnp.repeat(v_cache, rep, axis=1)
        scores = jnp.einsum("bhqd,bhkd->bhqk", q, k) * (Dh ** -0.5)
        p = _softmax(scores, axis=-1)
        o = jnp.einsum("bhqk,bhkd->bhqd", p, v)
        return (lambda x, *d: x.transpose(*d))(o, 0, 2, 1, 3).reshape(B, Sq, Hq * Dh) @ wo

    x = A_x
    g = _sigmoid((x * gate_w).sum(-1, keepdims=True))
    a = _A_ref(x, A_c_kv, A_w_q, A_w_uk, A_w_uv, A_w_o)
    b = _B_ref(x, B_k_cache, B_v_cache, B_wq, B_wo)
    return g * a + (1 - g) * b
```

```python
import jax
import jax.numpy as jnp
from jax import lax
import jax.experimental.pallas as pl
import jax.experimental.pallas.tpu as pltpu

BF16 = jnp.bfloat16
F32 = jnp.float32

H = 32
D = 128
S = 4096
M = 640
C = 512
HD = H * D
G = 4
NG = H // G
R = 8
SCALE = D ** -0.5

NT = (((1,), (1,)), ((), ()))
WO_CHUNKS = ((0, 26), (26, 5), (31, 1))


def _nt(a, b):
    return lax.dot_general(a, b, NT, preferred_element_type=F32)


def _nn(a, b):
    return jnp.dot(a, b, preferred_element_type=F32)


def _kernel(x_hbm, ckv_hbm, wqa_hbm, wuk_hbm, wuv_hbm, woa_hbm, k_hbm, v_hbm,
            wqb_hbm, wob_hbm, gw_hbm, out_hbm,
            x_buf, gw_buf, wqb_buf, wqa_buf, wuk_buf, ckv_buf, wuv_buf, woa_buf,
            k_buf, v_buf, wob_buf, g0_buf, q_scr, o_scr, out_buf,
            sem, ksem, vsem, wsem, osem):
    simple = [(x_hbm, x_buf), (gw_hbm, gw_buf), (wqb_hbm, wqb_buf),
              (wqa_hbm, wqa_buf), (wuk_hbm, wuk_buf), (ckv_hbm, ckv_buf),
              (wuv_hbm, wuv_buf), (woa_hbm, woa_buf)]

    def cp(i):
        src, dst = simple[i]
        return pltpu.make_async_copy(src, dst, sem.at[i])

    def cp_k(g):
        return pltpu.make_async_copy(k_hbm.at[pl.ds(g * G, G)],
                                     k_buf.at[pl.ds(g * G, G)], ksem.at[g])

    def cp_v(g):
        return pltpu.make_async_copy(v_hbm.at[pl.ds(g * G, G)],
                                     v_buf.at[pl.ds(g * G, G)], vsem.at[g])

    def cp_wo(i):
        s, n = WO_CHUNKS[i]
        return pltpu.make_async_copy(wob_hbm.at[pl.ds(s, n)],
                                     wob_buf.at[pl.ds(s, n)], wsem.at[i])

    for i in range(len(simple)):
        cp(i).start()
    for g in range(NG):
        cp_k(g).start()
        cp_v(g).start()
    for i in range(len(WO_CHUNKS)):
        cp_wo(i).start()

    row = lax.broadcasted_iota(jnp.int32, (HD, 128), 0)
    col = lax.broadcasted_iota(jnp.int32, (HD, 128), 1)
    g0_buf[...] = jnp.where((row >> 5) == col, 1.0, 0.0).astype(BF16)
    diag = ((lax.broadcasted_iota(jnp.int32, (H, HD), 1) & (H - 1))
            == lax.broadcasted_iota(jnp.int32, (H, HD), 0))

    def contract_major(coef, w2_ref):
        nb = coef.shape[1] // 128
        cs = jnp.concatenate([coef[:, b * 128:(b + 1) * 128] for b in range(nb)], axis=0)
        e = _nt(cs, g0_buf[...])
        acc = jnp.zeros((H, D), F32)
        for b in range(nb):
            sel = jnp.where(diag, e[b * H:(b + 1) * H], 0.0).astype(BF16)
            acc = acc + _nn(sel, w2_ref[b * HD:(b + 1) * HD, :])
        return acc

    def contract_minor(q, w2_ref, n):
        nb = n // 128
        ts = []
        for b in range(nb):
            t = _nt(q, w2_ref[b * HD:(b + 1) * HD, :])
            ts.append(jnp.where(diag, t, 0.0).astype(BF16))
        r = _nn(jnp.concatenate(ts, axis=0), g0_buf[...])
        return jnp.concatenate([r[b * H:(b + 1) * H] for b in range(nb)], axis=1)

    cp(0).wait()
    cp(1).wait()
    x = x_buf[0]
    gw = gw_buf[...].reshape(1, M)
    gate = jax.nn.sigmoid(jnp.sum(x.astype(F32) * gw.astype(F32), axis=-1, keepdims=True))

    cp(2).wait()
    qb = _nn(jnp.broadcast_to(x, (R, M)), wqb_buf[...]) * SCALE
    for h in range(H):
        q_scr[h] = qb[:, h * D:(h + 1) * D].astype(BF16)

    cp(3).wait()
    qa = contract_major(jnp.broadcast_to(x, (H, M)), wqa_buf) * SCALE
    cp(4).wait()
    qabs = contract_minor(qa.astype(BF16), wuk_buf, C)
    cp(5).wait()
    sa = _nt(qabs.astype(BF16), ckv_buf[...])
    ma = jnp.max(sa, axis=-1, keepdims=True)
    pa = jnp.exp(sa - ma)
    la = jnp.sum(pa, axis=-1, keepdims=True)
    ctxc = _nn(pa.astype(BF16), ckv_buf[...]) / la
    cp(6).wait()
    ctx = contract_major(ctxc.astype(BF16), wuv_buf)
    cp(7).wait()
    bd = ((lax.broadcasted_iota(jnp.int32, (H, HD), 1) >> 7)
          == lax.broadcasted_iota(jnp.int32, (H, HD), 0))
    cbd = jnp.where(bd, jnp.concatenate([ctx] * H, axis=1), 0.0).astype(BF16)
    out_a = jnp.sum(_nn(cbd, woa_buf[...]), axis=0, keepdims=True)

    def head(h, carry):
        @pl.when(h % G == 0)
        def _():
            cp_k(h // G).wait()
            cp_v(h // G).wait()
        s = _nt(q_scr[h], k_buf[h])
        m = jnp.max(s, axis=-1, keepdims=True)
        p = jnp.exp(s - m)
        l = jnp.sum(p, axis=-1, keepdims=True)
        o = _nn(p.astype(BF16), v_buf[h]) / l
        o_scr[h] = o.astype(BF16)
        return carry

    lax.fori_loop(0, H, head, 0)

    acc = jnp.zeros((R, M), F32)
    for i, (s0, n) in enumerate(WO_CHUNKS):
        cp_wo(i).wait()
        for h in range(s0, s0 + n):
            acc = acc + _nn(o_scr[h], wob_buf[h])
    out_b = acc[0:1]

    out = gate * out_a + (1.0 - gate) * out_b
    out_buf[0] = out.astype(BF16)
    ocp = pltpu.make_async_copy(out_buf, out_hbm, osem.at[0])
    ocp.start()
    ocp.wait()


@jax.jit
def pallas_gated_mix__compressed_kv_cla__gqa_block_cached__decode_kernel(
    A_x: jax.Array,
    A_c_kv: jax.Array,
    A_w_q: jax.Array,
    A_w_uk: jax.Array,
    A_w_uv: jax.Array,
    A_w_o: jax.Array,
    B_x: jax.Array,
    B_k_cache: jax.Array,
    B_v_cache: jax.Array,
    B_wq: jax.Array,
    B_wo: jax.Array,
    gate_w: jax.Array,
):
    del B_x
    args = (
        A_x,
        A_c_kv.reshape(S, C),
        A_w_q.reshape(M * H, D),
        A_w_uk.reshape(C * H, D),
        A_w_uv.reshape(C * H, D),
        A_w_o.reshape(HD, M),
        B_k_cache.reshape(H, S, D),
        B_v_cache.reshape(H, S, D),
        B_wq,
        B_wo.reshape(H, D, M),
        gate_w,
    )
    any_spec = pl.BlockSpec(memory_space=pl.ANY)
    scratch = [
        pltpu.VMEM((1, 1, M), BF16),
        pltpu.VMEM((M,), BF16),
        pltpu.VMEM((M, HD), BF16),
        pltpu.VMEM((M * H, D), BF16),
        pltpu.VMEM((C * H, D), BF16),
        pltpu.VMEM((S, C), BF16),
        pltpu.VMEM((C * H, D), BF16),
        pltpu.VMEM((HD, M), BF16),
        pltpu.VMEM((H, S, D), BF16),
        pltpu.VMEM((H, S, D), BF16),
        pltpu.VMEM((H, D, M), BF16),
        pltpu.VMEM((HD, 128), BF16),
        pltpu.VMEM((H, R, D), BF16),
        pltpu.VMEM((H, R, D), BF16),
        pltpu.VMEM((1, 1, M), BF16),
        pltpu.SemaphoreType.DMA((8,)),
        pltpu.SemaphoreType.DMA((NG,)),
        pltpu.SemaphoreType.DMA((NG,)),
        pltpu.SemaphoreType.DMA((len(WO_CHUNKS),)),
        pltpu.SemaphoreType.DMA((1,)),
    ]
    return pl.pallas_call(
        _kernel,
        out_shape=jax.ShapeDtypeStruct((1, 1, M), BF16),
        in_specs=[any_spec] * len(args),
        out_specs=any_spec,
        scratch_shapes=scratch,
        compiler_params=pltpu.CompilerParams(vmem_limit_bytes=120 * 1024 * 1024),
    )(*args)
```

```python
import jax
import jax.numpy as jnp
from jax import lax
import jax.experimental.pallas as pl
import jax.experimental.pallas.tpu as pltpu

BF16 = jnp.bfloat16
F32 = jnp.float32

H = 32
D = 128
S = 4096
M = 640
C = 512
HD = H * D
R = 8
SCALE = D ** -0.5

VH0 = 27
VPU_SIZES = (528, 96, 16)
WO_SIZES = (VH0 * D,) + VPU_SIZES
WO_STARTS = tuple(sum(WO_SIZES[:i]) for i in range(len(WO_SIZES)))
assert sum(WO_SIZES) == HD

_NT = (((1,), (1,)), ((), ()))


def _nt(a, b):
    return lax.dot_general(a, b, _NT, preferred_element_type=F32)


def _nn(a, b):
    return jnp.dot(a, b, preferred_element_type=F32)


def _kernel(x_hbm, ckv_hbm, wqa_hbm, wuk_hbm, wuv_hbm, woa_hbm, k_hbm, v_hbm,
            wqb_hbm, wob_hbm, gw_hbm, out_hbm,
            x_buf, gw_buf, wqb_buf, wqa_buf, wuk_buf, ckv_buf, wuv_buf, woa_buf,
            k_buf, v_buf, wo0_buf, wo1_buf, wo2_buf, wo3_buf,
            g0_buf, q_scr, p_scr, l_scr, o_scr, obc_scr, out_buf, sem):
    wo_bufs = (wo0_buf, wo1_buf, wo2_buf, wo3_buf)
    copies = [(x_hbm, x_buf), (gw_hbm, gw_buf), (wqb_hbm, wqb_buf), (k_hbm, k_buf),
              (wqa_hbm, wqa_buf), (wuk_hbm, wuk_buf), (ckv_hbm, ckv_buf),
              (v_hbm, v_buf), (wuv_hbm, wuv_buf), (woa_hbm, woa_buf)]
    for s0, n, buf in zip(WO_STARTS, WO_SIZES, wo_bufs):
        copies.append((wob_hbm.at[pl.ds(s0, n)], buf))
    X, GW, WQB, K, WQA, WUK, CKV, V, WUV, WOA, WOB = range(11)

    def cp(i):
        src, dst = copies[i]
        return pltpu.make_async_copy(src, dst, sem.at[i])

    for i in range(len(copies)):
        cp(i).start()

    row = lax.broadcasted_iota(jnp.int32, (HD, 128), 0)
    col = lax.broadcasted_iota(jnp.int32, (HD, 128), 1)
    g0_buf[...] = jnp.where((row >> 5) == col, 1.0, 0.0).astype(BF16)
    diag = ((lax.broadcasted_iota(jnp.int32, (H, HD), 1) & (H - 1))
            == lax.broadcasted_iota(jnp.int32, (H, HD), 0))

    def contract_major(coef, w2_ref):
        nb = coef.shape[1] // 128
        cs = jnp.concatenate([coef[:, b * 128:(b + 1) * 128] for b in range(nb)], axis=0)
        e = _nt(cs, g0_buf[...])
        acc = jnp.zeros((H, D), F32)
        for b in range(nb):
            sel = jnp.where(diag, e[b * H:(b + 1) * H], 0.0).astype(BF16)
            acc = acc + _nn(sel, w2_ref[b * HD:(b + 1) * HD, :])
        return acc

    def contract_minor(q, w2_ref, n):
        nb = n // 128
        ts = []
        for b in range(nb):
            t = _nt(q, w2_ref[b * HD:(b + 1) * HD, :])
            ts.append(jnp.where(diag, t, 0.0).astype(BF16))
        r = _nn(jnp.concatenate(ts, axis=0), g0_buf[...])
        return jnp.concatenate([r[b * H:(b + 1) * H] for b in range(nb)], axis=1)

    cp(X).wait()
    cp(GW).wait()
    x = x_buf[0]
    gw = gw_buf[...].reshape(1, M)
    gate = jax.nn.sigmoid(
        jnp.sum(x.astype(F32) * gw.astype(F32), axis=-1, keepdims=True))

    cp(WQB).wait()
    qb = _nn(jnp.broadcast_to(x, (R, M)), wqb_buf[...]) * SCALE
    for h in range(H):
        q_scr[h] = qb[:, h * D:(h + 1) * D].astype(BF16)

    cp(K).wait()

    def qk_head(h, carry):
        s = _nt(q_scr[h], k_buf[h])
        m = jnp.max(s, axis=-1, keepdims=True)
        p = jnp.exp(s - m)
        l_scr[h] = jnp.broadcast_to(jnp.sum(p, axis=-1, keepdims=True), (R, D))
        p_scr[h] = p.astype(BF16)
        return carry

    lax.fori_loop(0, H, qk_head, 0)

    cp(WQA).wait()
    qa = contract_major(jnp.broadcast_to(x, (H, M)), wqa_buf) * SCALE
    cp(WUK).wait()
    qabs = contract_minor(qa.astype(BF16), wuk_buf, C)
    cp(CKV).wait()
    sa = _nt(qabs.astype(BF16), ckv_buf[...])
    ma = jnp.max(sa, axis=-1, keepdims=True)
    pa = jnp.exp(sa - ma)
    la = jnp.sum(pa, axis=-1, keepdims=True)
    ctxc = _nn(pa.astype(BF16), ckv_buf[...]) / la

    cp(V).wait()

    def pv_head(h, carry):
        o_scr[h] = _nn(p_scr[h], v_buf[h]) / l_scr[h]
        return carry

    lax.fori_loop(0, H, pv_head, 0)
    for h in range(VH0, H):
        o_h = o_scr[h][0:1] * (1.0 - gate)
        obc_scr[(h - VH0) * D:(h - VH0 + 1) * D, :] = jnp.broadcast_to(o_h, (D, D)).T

    cp(WUV).wait()
    ctx = contract_major(ctxc.astype(BF16), wuv_buf)
    cp(WOA).wait()
    bd = ((lax.broadcasted_iota(jnp.int32, (H, HD), 1) >> 7)
          == lax.broadcasted_iota(jnp.int32, (H, HD), 0))
    cbd = jnp.where(bd, jnp.concatenate([ctx] * H, axis=1), 0.0).astype(BF16)
    out_a = jnp.sum(_nn(cbd, woa_buf[...]), axis=0, keepdims=True)

    cp(WOB).wait()
    acc = jnp.zeros((R, M), F32)
    for h in range(VH0):
        acc = acc + _nn(o_scr[h].astype(BF16), wo0_buf[h * D:(h + 1) * D, :])
    base = gate * out_a + (1.0 - gate) * acc[0:1]
    sub = lax.broadcasted_iota(jnp.int32, (R, M), 0)
    acc8 = jnp.where(sub == 0, jnp.broadcast_to(base, (R, M)), 0.0)
    r0 = 0
    for i, n in enumerate(VPU_SIZES):
        cp(WOB + 1 + i).wait()
        for r in range(0, n, 16):
            w = wo_bufs[1 + i][r:r + 16, :].astype(F32)
            ob = jnp.concatenate([obc_scr[r0 + r:r0 + r + 16, :]] * (M // D), axis=1)
            pr = w * ob
            acc8 = acc8 + pr[0:8] + pr[8:16]
        r0 += n

    out_buf[0] = jnp.sum(acc8, axis=0, keepdims=True).astype(BF16)
    out_cp = pltpu.make_async_copy(out_buf, out_hbm, sem.at[len(copies)])
    out_cp.start()
    out_cp.wait()


@jax.jit
def pallas_gated_mix__compressed_kv_cla__gqa_block_cached__decode_kernel(
    A_x: jax.Array,
    A_c_kv: jax.Array,
    A_w_q: jax.Array,
    A_w_uk: jax.Array,
    A_w_uv: jax.Array,
    A_w_o: jax.Array,
    B_x: jax.Array,
    B_k_cache: jax.Array,
    B_v_cache: jax.Array,
    B_wq: jax.Array,
    B_wo: jax.Array,
    gate_w: jax.Array,
):
    del B_x
    args = (
        A_x,
        A_c_kv.reshape(S, C),
        A_w_q.reshape(M * H, D),
        A_w_uk.reshape(C * H, D),
        A_w_uv.reshape(C * H, D),
        A_w_o.reshape(HD, M),
        B_k_cache.reshape(H, S, D),
        B_v_cache.reshape(H, S, D),
        B_wq,
        B_wo,
        gate_w,
    )
    any_spec = pl.BlockSpec(memory_space=pl.ANY)
    scratch = [
        pltpu.VMEM((1, 1, M), BF16),
        pltpu.VMEM((M,), BF16),
        pltpu.VMEM((M, HD), BF16),
        pltpu.VMEM((M * H, D), BF16),
        pltpu.VMEM((C * H, D), BF16),
        pltpu.VMEM((S, C), BF16),
        pltpu.VMEM((C * H, D), BF16),
        pltpu.VMEM((HD, M), BF16),
        pltpu.VMEM((H, S, D), BF16),
        pltpu.VMEM((H, S, D), BF16),
    ] + [pltpu.VMEM((n, M), BF16) for n in WO_SIZES] + [
        pltpu.VMEM((HD, 128), BF16),
        pltpu.VMEM((H, R, D), BF16),
        pltpu.VMEM((H, R, S), BF16),
        pltpu.VMEM((H, R, D), F32),
        pltpu.VMEM((H, R, D), F32),
        pltpu.VMEM(((H - VH0) * D, D), F32),
        pltpu.VMEM((1, 1, M), BF16),
        pltpu.SemaphoreType.DMA((10 + len(WO_SIZES) + 1,)),
    ]
    return pl.pallas_call(
        _kernel,
        out_shape=jax.ShapeDtypeStruct((1, 1, M), BF16),
        in_specs=[any_spec] * len(args),
        out_specs=any_spec,
        scratch_shapes=scratch,
        compiler_params=pltpu.CompilerParams(vmem_limit_bytes=120 * 1024 * 1024),
    )(*args)
```

```python
import jax
import jax.numpy as jnp
from jax import lax
import jax.experimental.pallas as pl
import jax.experimental.pallas.tpu as pltpu

BF16 = jnp.bfloat16
F32 = jnp.float32

H = 32
D = 128
S = 4096
M = 640
C = 512
HD = H * D
R = 8
SCALE = D ** -0.5

MXU_HEADS = (16, 11)
VPU_ROWS = (256, 128, 96, 64, 48, 32, 16)
VH0 = sum(MXU_HEADS)
WO_SIZES = tuple(n * D for n in MXU_HEADS) + VPU_ROWS
WO_STARTS = tuple(sum(WO_SIZES[:i]) for i in range(len(WO_SIZES)))
assert sum(WO_SIZES) == HD
N_WHOLE = 10

_NT = (((1,), (1,)), ((), ()))


def _nt(a, b):
    return lax.dot_general(a, b, _NT, preferred_element_type=F32)


def _nn(a, b):
    return jnp.dot(a, b, preferred_element_type=F32)


def _kernel(x_hbm, ckv_hbm, wqa_hbm, wuk_hbm, wuv_hbm, woa_hbm, k_hbm, v_hbm,
            wqb_hbm, wob_hbm, gw_hbm, out_hbm,
            x_buf, gw_buf, wqb_buf, wqa_buf, wuk_buf, ckv_buf, wuv_buf, woa_buf,
            k_buf, v_buf, *rest):
    wo_bufs = rest[:len(WO_SIZES)]
    g0_buf, q_scr, p_scr, l_scr, o_scr, obc_scr, out_buf, sem = rest[len(WO_SIZES):]

    copies = [(x_hbm, x_buf), (gw_hbm, gw_buf), (wqb_hbm, wqb_buf), (k_hbm, k_buf),
              (wqa_hbm, wqa_buf), (wuk_hbm, wuk_buf), (ckv_hbm, ckv_buf),
              (v_hbm, v_buf), (wuv_hbm, wuv_buf), (woa_hbm, woa_buf)]
    for s0, n, buf in zip(WO_STARTS, WO_SIZES, wo_bufs):
        copies.append((wob_hbm.at[pl.ds(s0, n)], buf))
    X, GW, WQB, K, WQA, WUK, CKV, V, WUV, WOA, WOB = range(N_WHOLE + 1)

    def cp(i):
        src, dst = copies[i]
        return pltpu.make_async_copy(src, dst, sem.at[i])

    for i in range(len(copies)):
        cp(i).start()

    row = lax.broadcasted_iota(jnp.int32, (HD, 128), 0)
    col = lax.broadcasted_iota(jnp.int32, (HD, 128), 1)
    g0_buf[...] = jnp.where((row >> 5) == col, 1.0, 0.0).astype(BF16)
    diag = ((lax.broadcasted_iota(jnp.int32, (H, HD), 1) & (H - 1))
            == lax.broadcasted_iota(jnp.int32, (H, HD), 0))

    def contract_major(coef, w2_ref):
        nb = coef.shape[1] // 128
        cs = jnp.concatenate([coef[:, b * 128:(b + 1) * 128] for b in range(nb)], axis=0)
        e = _nt(cs, g0_buf[...])
        acc = jnp.zeros((H, D), F32)
        for b in range(nb):
            sel = jnp.where(diag, e[b * H:(b + 1) * H], 0.0).astype(BF16)
            acc = acc + _nn(sel, w2_ref[b * HD:(b + 1) * HD, :])
        return acc

    def contract_minor(q, w2_ref, n):
        nb = n // 128
        ts = []
        for b in range(nb):
            t = _nt(q, w2_ref[b * HD:(b + 1) * HD, :])
            ts.append(jnp.where(diag, t, 0.0).astype(BF16))
        r = _nn(jnp.concatenate(ts, axis=0), g0_buf[...])
        return jnp.concatenate([r[b * H:(b + 1) * H] for b in range(nb)], axis=1)

    cp(X).wait()
    cp(GW).wait()
    x = x_buf[0]
    gw = gw_buf[...].reshape(1, M)
    gate = jax.nn.sigmoid(
        jnp.sum(x.astype(F32) * gw.astype(F32), axis=-1, keepdims=True))

    cp(WQB).wait()
    qb = _nn(jnp.broadcast_to(x, (R, M)), wqb_buf[...]) * SCALE
    for h in range(H):
        q_scr[h] = qb[:, h * D:(h + 1) * D].astype(BF16)

    cp(K).wait()

    def qk_head(h, carry):
        s = _nt(q_scr[h], k_buf[h])
        m = jnp.max(s, axis=-1, keepdims=True)
        p = jnp.exp(s - m)
        l_scr[h] = jnp.broadcast_to(jnp.sum(p, axis=-1, keepdims=True), (R, D))
        p_scr[h] = p.astype(BF16)
        return carry

    lax.fori_loop(0, H, qk_head, 0)

    cp(WQA).wait()
    qa = contract_major(jnp.broadcast_to(x, (H, M)), wqa_buf) * SCALE
    cp(WUK).wait()
    qabs = contract_minor(qa.astype(BF16), wuk_buf, C)
    cp(CKV).wait()
    sa = _nt(qabs.astype(BF16), ckv_buf[...])
    ma = jnp.max(sa, axis=-1, keepdims=True)
    pa = jnp.exp(sa - ma)
    la = jnp.sum(pa, axis=-1, keepdims=True)
    ctxc = _nn(pa.astype(BF16), ckv_buf[...]) / la

    cp(V).wait()

    def pv_head(h, carry):
        o_scr[h] = _nn(p_scr[h], v_buf[h]) / l_scr[h]
        return carry

    lax.fori_loop(0, H, pv_head, 0)
    for h in range(VH0, H):
        o_h = o_scr[h][0:1] * (1.0 - gate)
        obc_scr[(h - VH0) * D:(h - VH0 + 1) * D, :] = jnp.broadcast_to(o_h, (D, D)).T

    cp(WUV).wait()
    ctx = contract_major(ctxc.astype(BF16), wuv_buf)
    cp(WOA).wait()
    bd = ((lax.broadcasted_iota(jnp.int32, (H, HD), 1) >> 7)
          == lax.broadcasted_iota(jnp.int32, (H, HD), 0))
    cbd = jnp.where(bd, jnp.concatenate([ctx] * H, axis=1), 0.0).astype(BF16)
    out_a = jnp.sum(_nn(cbd, woa_buf[...]), axis=0, keepdims=True)

    acc = jnp.zeros((R, M), F32)
    h0 = 0
    for i, nh in enumerate(MXU_HEADS):
        cp(WOB + i).wait()
        for h in range(nh):
            acc = acc + _nn(o_scr[h0 + h].astype(BF16), wo_bufs[i][h * D:(h + 1) * D, :])
        h0 += nh
    base = gate * out_a + (1.0 - gate) * acc[0:1]
    sub = lax.broadcasted_iota(jnp.int32, (R, M), 0)
    acc8 = jnp.where(sub == 0, jnp.broadcast_to(base, (R, M)), 0.0)
    r0 = 0
    for i, n in enumerate(VPU_ROWS):
        j = len(MXU_HEADS) + i
        cp(WOB + j).wait()
        for r in range(0, n, 16):
            w = wo_bufs[j][r:r + 16, :].astype(F32)
            ob = jnp.concatenate([obc_scr[r0 + r:r0 + r + 16, :]] * (M // D), axis=1)
            pr = w * ob
            acc8 = acc8 + pr[0:8] + pr[8:16]
        r0 += n

    out_buf[0] = jnp.sum(acc8, axis=0, keepdims=True).astype(BF16)
    out_cp = pltpu.make_async_copy(out_buf, out_hbm, sem.at[len(copies)])
    out_cp.start()
    out_cp.wait()


@jax.jit
def pallas_gated_mix__compressed_kv_cla__gqa_block_cached__decode_kernel(
    A_x: jax.Array,
    A_c_kv: jax.Array,
    A_w_q: jax.Array,
    A_w_uk: jax.Array,
    A_w_uv: jax.Array,
    A_w_o: jax.Array,
    B_x: jax.Array,
    B_k_cache: jax.Array,
    B_v_cache: jax.Array,
    B_wq: jax.Array,
    B_wo: jax.Array,
    gate_w: jax.Array,
):
    del B_x
    args = (
        A_x,
        A_c_kv.reshape(S, C),
        A_w_q.reshape(M * H, D),
        A_w_uk.reshape(C * H, D),
        A_w_uv.reshape(C * H, D),
        A_w_o.reshape(HD, M),
        B_k_cache.reshape(H, S, D),
        B_v_cache.reshape(H, S, D),
        B_wq,
        B_wo,
        gate_w,
    )
    any_spec = pl.BlockSpec(memory_space=pl.ANY)
    scratch = [
        pltpu.VMEM((1, 1, M), BF16),
        pltpu.VMEM((M,), BF16),
        pltpu.VMEM((M, HD), BF16),
        pltpu.VMEM((M * H, D), BF16),
        pltpu.VMEM((C * H, D), BF16),
        pltpu.VMEM((S, C), BF16),
        pltpu.VMEM((C * H, D), BF16),
        pltpu.VMEM((HD, M), BF16),
        pltpu.VMEM((H, S, D), BF16),
        pltpu.VMEM((H, S, D), BF16),
    ] + [pltpu.VMEM((n, M), BF16) for n in WO_SIZES] + [
        pltpu.VMEM((HD, 128), BF16),
        pltpu.VMEM((H, R, D), BF16),
        pltpu.VMEM((H, R, S), BF16),
        pltpu.VMEM((H, R, D), F32),
        pltpu.VMEM((H, R, D), F32),
        pltpu.VMEM(((H - VH0) * D, D), F32),
        pltpu.VMEM((1, 1, M), BF16),
        pltpu.SemaphoreType.DMA((N_WHOLE + len(WO_SIZES) + 1,)),
    ]
    return pl.pallas_call(
        _kernel,
        out_shape=jax.ShapeDtypeStruct((1, 1, M), BF16),
        in_specs=[any_spec] * len(args),
        out_specs=any_spec,
        scratch_shapes=scratch,
        compiler_params=pltpu.CompilerParams(
            vmem_limit_bytes=120 * 1024 * 1024,
            disable_semaphore_checks=True,
        ),
    )(*args)
```

```python
import jax
import jax.numpy as jnp
from jax import lax
import jax.experimental.pallas as pl
import jax.experimental.pallas.tpu as pltpu

BF16 = jnp.bfloat16
F32 = jnp.float32

H = 32
D = 128
S = 4096
M = 640
C = 512
HD = H * D
R = 8
SCALE = D ** -0.5

MXU_HEADS = (16, 11)
VPU_ROWS = (256, 128, 96, 64, 48, 32, 16)
VH0 = sum(MXU_HEADS)
WO_SIZES = tuple(n * D for n in MXU_HEADS) + VPU_ROWS
WO_STARTS = tuple(sum(WO_SIZES[:i]) for i in range(len(WO_SIZES)))
assert sum(WO_SIZES) == HD
N_WHOLE = 10

_NT = (((1,), (1,)), ((), ()))


def _nt(a, b):
    return lax.dot_general(a, b, _NT, preferred_element_type=F32)


def _nn(a, b):
    return jnp.dot(a, b, preferred_element_type=F32)


def _kernel(x_hbm, ckv_hbm, wqa_hbm, wuk_hbm, wuv_hbm, woa_hbm, k_hbm, v_hbm,
            wqb_hbm, wob_hbm, gw_hbm, out_hbm,
            x_buf, gw_buf, wqb_buf, wqa_buf, wuk_buf, ckv_buf, wuv_buf, woa_buf,
            k_buf, v_buf, *rest):
    wo_bufs = rest[:len(WO_SIZES)]
    g0_buf, q_scr, p_scr, l_scr, o_scr, obc_scr, out_buf, sem = rest[len(WO_SIZES):]

    copies = [(x_hbm, x_buf), (gw_hbm, gw_buf), (wqb_hbm, wqb_buf), (k_hbm, k_buf),
              (wqa_hbm, wqa_buf), (wuk_hbm, wuk_buf), (ckv_hbm, ckv_buf),
              (v_hbm, v_buf), (wuv_hbm, wuv_buf), (woa_hbm, woa_buf)]
    for s0, n, buf in zip(WO_STARTS, WO_SIZES, wo_bufs):
        copies.append((wob_hbm.at[pl.ds(s0, n)], buf))
    X, GW, WQB, K, WQA, WUK, CKV, V, WUV, WOA, WOB = range(N_WHOLE + 1)

    def cp(i):
        src, dst = copies[i]
        return pltpu.make_async_copy(src, dst, sem.at[i])

    for i in range(len(copies)):
        cp(i).start()

    row = lax.broadcasted_iota(jnp.int32, (HD, 128), 0)
    col = lax.broadcasted_iota(jnp.int32, (HD, 128), 1)
    g0_buf[...] = jnp.where((row >> 5) == col, 1.0, 0.0).astype(BF16)
    diag = ((lax.broadcasted_iota(jnp.int32, (H, HD), 1) & (H - 1))
            == lax.broadcasted_iota(jnp.int32, (H, HD), 0))

    def contract_major(coef, w2_ref):
        nb = coef.shape[1] // 128
        cs = jnp.concatenate([coef[:, b * 128:(b + 1) * 128] for b in range(nb)], axis=0)
        e = _nt(cs, g0_buf[...])
        acc = jnp.zeros((H, D), F32)
        for b in range(nb):
            sel = jnp.where(diag, e[b * H:(b + 1) * H], 0.0).astype(BF16)
            acc = acc + _nn(sel, w2_ref[b * HD:(b + 1) * HD, :])
        return acc

    def contract_minor(q, w2_ref, n):
        nb = n // 128
        ts = []
        for b in range(nb):
            t = _nt(q, w2_ref[b * HD:(b + 1) * HD, :])
            ts.append(jnp.where(diag, t, 0.0).astype(BF16))
        r = _nn(jnp.concatenate(ts, axis=0), g0_buf[...])
        return jnp.concatenate([r[b * H:(b + 1) * H] for b in range(nb)], axis=1)

    cp(X).wait()
    cp(GW).wait()
    x = x_buf[0]
    gw = gw_buf[...].reshape(1, M)
    gate = jax.nn.sigmoid(
        jnp.sum(x.astype(F32) * gw.astype(F32), axis=-1, keepdims=True))

    cp(WQB).wait()
    qb = _nn(jnp.broadcast_to(x, (R, M)), wqb_buf[...]) * SCALE
    for h in range(H):
        q_scr[h] = qb[:, h * D:(h + 1) * D].astype(BF16)

    cp(K).wait()

    def qk_head(h, carry):
        s = _nt(q_scr[h], k_buf[h])
        m = jnp.max(s, axis=-1, keepdims=True)
        p = jnp.exp(s - m)
        l_scr[h] = jnp.broadcast_to(jnp.sum(p, axis=-1, keepdims=True), (R, D))
        p_scr[h] = p.astype(BF16)
        return carry

    lax.fori_loop(0, H, qk_head, 0)

    cp(WQA).wait()
    qa = contract_major(jnp.broadcast_to(x, (H, M)), wqa_buf) * SCALE
    cp(WUK).wait()
    qabs = contract_minor(qa.astype(BF16), wuk_buf, C)
    cp(CKV).wait()
    sa = _nt(qabs.astype(BF16), ckv_buf[...])
    ma = jnp.max(sa, axis=-1, keepdims=True)
    pa = jnp.exp(sa - ma)
    la = jnp.sum(pa, axis=-1, keepdims=True)
    ctxc = _nn(pa.astype(BF16), ckv_buf[...]) / la

    cp(V).wait()

    def pv_head(h, carry):
        o_scr[h] = _nn(p_scr[h], v_buf[h]) / l_scr[h]
        return carry

    lax.fori_loop(0, H, pv_head, 0)
    for h in range(VH0, H):
        o_h = o_scr[h][0:1] * (1.0 - gate)
        obc_scr[(h - VH0) * D:(h - VH0 + 1) * D, :] = jnp.broadcast_to(o_h, (D, D)).T

    cp(WUV).wait()
    ctx = contract_major(ctxc.astype(BF16), wuv_buf)
    cp(WOA).wait()
    bd = ((lax.broadcasted_iota(jnp.int32, (H, HD), 1) >> 7)
          == lax.broadcasted_iota(jnp.int32, (H, HD), 0))
    cbd = jnp.where(bd, jnp.concatenate([ctx] * H, axis=1), 0.0).astype(BF16)
    out_a = jnp.sum(_nn(cbd, woa_buf[...]), axis=0, keepdims=True)

    acc = jnp.zeros((R, M), F32)
    h0 = 0
    for i, nh in enumerate(MXU_HEADS):
        cp(WOB + i).wait()
        for h in range(nh):
            acc = acc + _nn(o_scr[h0 + h].astype(BF16), wo_bufs[i][h * D:(h + 1) * D, :])
        h0 += nh
    base = gate * out_a + (1.0 - gate) * acc[0:1]
    sub = lax.broadcasted_iota(jnp.int32, (R, M), 0)
    acc8 = jnp.where(sub == 0, jnp.broadcast_to(base, (R, M)), 0.0)
    r0 = 0
    for i, n in enumerate(VPU_ROWS):
        j = len(MXU_HEADS) + i
        cp(WOB + j).wait()
        for r in range(0, n, 16):
            w = wo_bufs[j][r:r + 16, :].astype(F32)
            ob = jnp.concatenate([obc_scr[r0 + r:r0 + r + 16, :]] * (M // D), axis=1)
            pr = w * ob
            acc8 = acc8 + pr[0:8] + pr[8:16]
        r0 += n

    out_buf[0] = jnp.sum(acc8, axis=0, keepdims=True).astype(BF16)
    out_cp = pltpu.make_async_copy(out_buf, out_hbm, sem.at[len(copies)])
    out_cp.start()
    out_cp.wait()


@jax.jit
def pallas_gated_mix__compressed_kv_cla__gqa_block_cached__decode_kernel(
    A_x: jax.Array,
    A_c_kv: jax.Array,
    A_w_q: jax.Array,
    A_w_uk: jax.Array,
    A_w_uv: jax.Array,
    A_w_o: jax.Array,
    B_x: jax.Array,
    B_k_cache: jax.Array,
    B_v_cache: jax.Array,
    B_wq: jax.Array,
    B_wo: jax.Array,
    gate_w: jax.Array,
):
    del B_x
    args = (
        A_x,
        A_c_kv.reshape(S, C),
        A_w_q.reshape(M * H, D),
        A_w_uk.reshape(C * H, D),
        A_w_uv.reshape(C * H, D),
        A_w_o.reshape(HD, M),
        B_k_cache.reshape(H, S, D),
        B_v_cache.reshape(H, S, D),
        B_wq,
        B_wo,
        gate_w,
    )
    any_spec = pl.BlockSpec(memory_space=pl.ANY)
    scratch = [
        pltpu.VMEM((1, 1, M), BF16),
        pltpu.VMEM((M,), BF16),
        pltpu.VMEM((M, HD), BF16),
        pltpu.VMEM((M * H, D), BF16),
        pltpu.VMEM((C * H, D), BF16),
        pltpu.VMEM((S, C), BF16),
        pltpu.VMEM((C * H, D), BF16),
        pltpu.VMEM((HD, M), BF16),
        pltpu.VMEM((H, S, D), BF16),
        pltpu.VMEM((H, S, D), BF16),
    ] + [pltpu.VMEM((n, M), BF16) for n in WO_SIZES] + [
        pltpu.VMEM((HD, 128), BF16),
        pltpu.VMEM((H, R, D), BF16),
        pltpu.VMEM((H, R, S), BF16),
        pltpu.VMEM((H, R, D), F32),
        pltpu.VMEM((H, R, D), F32),
        pltpu.VMEM(((H - VH0) * D, D), F32),
        pltpu.VMEM((1, 1, M), BF16),
        pltpu.SemaphoreType.DMA((N_WHOLE + len(WO_SIZES) + 1,)),
    ]
    params = dict(vmem_limit_bytes=120 * 1024 * 1024)
    if hasattr(pltpu.CompilerParams, "disable_semaphore_checks"):
        params["disable_semaphore_checks"] = True
    return pl.pallas_call(
        _kernel,
        out_shape=jax.ShapeDtypeStruct((1, 1, M), BF16),
        in_specs=[any_spec] * len(args),
        out_specs=any_spec,
        scratch_shapes=scratch,
        compiler_params=pltpu.CompilerParams(**params),
    )(*args)
```

```python
import jax
import jax.numpy as jnp
from jax import lax
import jax.experimental.pallas as pl
import jax.experimental.pallas.tpu as pltpu

BF16 = jnp.bfloat16
F32 = jnp.float32

H = 32
D = 128
S = 4096
M = 640
C = 512
HD = H * D
R = 8
SCALE = D ** -0.5

MXU_HEADS = (16, 11)
VPU_ROWS = (256, 128, 96, 64, 48, 32, 16)
VH0 = sum(MXU_HEADS)
WO_SIZES = tuple(n * D for n in MXU_HEADS) + VPU_ROWS
WO_STARTS = tuple(sum(WO_SIZES[:i]) for i in range(len(WO_SIZES)))
assert sum(WO_SIZES) == HD
N_WHOLE = 10

_NT = (((1,), (1,)), ((), ()))


def _nt(a, b):
    return lax.dot_general(a, b, _NT, preferred_element_type=F32)


def _nn(a, b):
    return jnp.dot(a, b, preferred_element_type=F32)


def _kernel(*refs):
    pl.run_scoped(lambda sem: _body(sem, *refs),
                  pltpu.SemaphoreType.DMA((N_WHOLE + len(WO_SIZES) + 1,)))


def _body(sem, x_hbm, ckv_hbm, wqa_hbm, wuk_hbm, wuv_hbm, woa_hbm, k_hbm, v_hbm,
          wqb_hbm, wob_hbm, gw_hbm, out_hbm,
          x_buf, gw_buf, wqb_buf, wqa_buf, wuk_buf, ckv_buf, wuv_buf, woa_buf,
          k_buf, v_buf, *rest):
    wo_bufs = rest[:len(WO_SIZES)]
    g0_buf, q_scr, p_scr, l_scr, o_scr, obc_scr, out_buf = rest[len(WO_SIZES):]

    copies = [(x_hbm, x_buf), (gw_hbm, gw_buf), (wqb_hbm, wqb_buf), (k_hbm, k_buf),
              (wqa_hbm, wqa_buf), (wuk_hbm, wuk_buf), (ckv_hbm, ckv_buf),
              (v_hbm, v_buf), (wuv_hbm, wuv_buf), (woa_hbm, woa_buf)]
    for s0, n, buf in zip(WO_STARTS, WO_SIZES, wo_bufs):
        copies.append((wob_hbm.at[pl.ds(s0, n)], buf))
    X, GW, WQB, K, WQA, WUK, CKV, V, WUV, WOA, WOB = range(N_WHOLE + 1)

    def cp(i):
        src, dst = copies[i]
        return pltpu.make_async_copy(src, dst, sem.at[i])

    for i in range(len(copies)):
        cp(i).start()

    row = lax.broadcasted_iota(jnp.int32, (HD, 128), 0)
    col = lax.broadcasted_iota(jnp.int32, (HD, 128), 1)
    g0_buf[...] = jnp.where((row >> 5) == col, 1.0, 0.0).astype(BF16)
    diag = ((lax.broadcasted_iota(jnp.int32, (H, HD), 1) & (H - 1))
            == lax.broadcasted_iota(jnp.int32, (H, HD), 0))

    def contract_major(coef, w2_ref):
        nb = coef.shape[1] // 128
        cs = jnp.concatenate([coef[:, b * 128:(b + 1) * 128] for b in range(nb)], axis=0)
        e = _nt(cs, g0_buf[...])
        acc = jnp.zeros((H, D), F32)
        for b in range(nb):
            sel = jnp.where(diag, e[b * H:(b + 1) * H], 0.0).astype(BF16)
            acc = acc + _nn(sel, w2_ref[b * HD:(b + 1) * HD, :])
        return acc

    def contract_minor(q, w2_ref, n):
        nb = n // 128
        ts = []
        for b in range(nb):
            t = _nt(q, w2_ref[b * HD:(b + 1) * HD, :])
            ts.append(jnp.where(diag, t, 0.0).astype(BF16))
        r = _nn(jnp.concatenate(ts, axis=0), g0_buf[...])
        return jnp.concatenate([r[b * H:(b + 1) * H] for b in range(nb)], axis=1)

    cp(X).wait()
    cp(GW).wait()
    x = x_buf[0]
    gw = gw_buf[...].reshape(1, M)
    gate = jax.nn.sigmoid(
        jnp.sum(x.astype(F32) * gw.astype(F32), axis=-1, keepdims=True))

    cp(WQB).wait()
    qb = _nn(jnp.broadcast_to(x, (R, M)), wqb_buf[...]) * SCALE
    for h in range(H):
        q_scr[h] = qb[:, h * D:(h + 1) * D].astype(BF16)

    cp(K).wait()

    def qk_head(h, carry):
        s = _nt(q_scr[h], k_buf[h])
        m = jnp.max(s, axis=-1, keepdims=True)
        p = jnp.exp(s - m)
        l_scr[h] = jnp.broadcast_to(jnp.sum(p, axis=-1, keepdims=True), (R, D))
        p_scr[h] = p.astype(BF16)
        return carry

    lax.fori_loop(0, H, qk_head, 0)

    cp(WQA).wait()
    qa = contract_major(jnp.broadcast_to(x, (H, M)), wqa_buf) * SCALE
    cp(WUK).wait()
    qabs = contract_minor(qa.astype(BF16), wuk_buf, C)
    cp(CKV).wait()
    sa = _nt(qabs.astype(BF16), ckv_buf[...])
    ma = jnp.max(sa, axis=-1, keepdims=True)
    pa = jnp.exp(sa - ma)
    la = jnp.sum(pa, axis=-1, keepdims=True)
    ctxc = _nn(pa.astype(BF16), ckv_buf[...]) / la

    cp(V).wait()

    def pv_head(h, carry):
        o_scr[h] = _nn(p_scr[h], v_buf[h]) / l_scr[h]
        return carry

    lax.fori_loop(0, H, pv_head, 0)
    for h in range(VH0, H):
        o_h = o_scr[h][0:1] * (1.0 - gate)
        obc_scr[(h - VH0) * D:(h - VH0 + 1) * D, :] = jnp.broadcast_to(o_h, (D, D)).T

    cp(WUV).wait()
    ctx = contract_major(ctxc.astype(BF16), wuv_buf)
    cp(WOA).wait()
    bd = ((lax.broadcasted_iota(jnp.int32, (H, HD), 1) >> 7)
          == lax.broadcasted_iota(jnp.int32, (H, HD), 0))
    cbd = jnp.where(bd, jnp.concatenate([ctx] * H, axis=1), 0.0).astype(BF16)
    out_a = jnp.sum(_nn(cbd, woa_buf[...]), axis=0, keepdims=True)

    acc = jnp.zeros((R, M), F32)
    h0 = 0
    for i, nh in enumerate(MXU_HEADS):
        cp(WOB + i).wait()
        for h in range(nh):
            acc = acc + _nn(o_scr[h0 + h].astype(BF16), wo_bufs[i][h * D:(h + 1) * D, :])
        h0 += nh
    base = gate * out_a + (1.0 - gate) * acc[0:1]
    sub = lax.broadcasted_iota(jnp.int32, (R, M), 0)
    acc8 = jnp.where(sub == 0, jnp.broadcast_to(base, (R, M)), 0.0)
    r0 = 0
    for i, n in enumerate(VPU_ROWS):
        j = len(MXU_HEADS) + i
        cp(WOB + j).wait()
        for r in range(0, n, 16):
            w = wo_bufs[j][r:r + 16, :].astype(F32)
            ob = jnp.concatenate([obc_scr[r0 + r:r0 + r + 16, :]] * (M // D), axis=1)
            pr = w * ob
            acc8 = acc8 + pr[0:8] + pr[8:16]
        r0 += n

    out_buf[0] = jnp.sum(acc8, axis=0, keepdims=True).astype(BF16)
    out_cp = pltpu.make_async_copy(out_buf, out_hbm, sem.at[len(copies)])
    out_cp.start()
    out_cp.wait()


@jax.jit
def pallas_gated_mix__compressed_kv_cla__gqa_block_cached__decode_kernel(
    A_x: jax.Array,
    A_c_kv: jax.Array,
    A_w_q: jax.Array,
    A_w_uk: jax.Array,
    A_w_uv: jax.Array,
    A_w_o: jax.Array,
    B_x: jax.Array,
    B_k_cache: jax.Array,
    B_v_cache: jax.Array,
    B_wq: jax.Array,
    B_wo: jax.Array,
    gate_w: jax.Array,
):
    del B_x
    args = (
        A_x,
        A_c_kv.reshape(S, C),
        A_w_q.reshape(M * H, D),
        A_w_uk.reshape(C * H, D),
        A_w_uv.reshape(C * H, D),
        A_w_o.reshape(HD, M),
        B_k_cache.reshape(H, S, D),
        B_v_cache.reshape(H, S, D),
        B_wq,
        B_wo,
        gate_w,
    )
    any_spec = pl.BlockSpec(memory_space=pl.ANY)
    scratch = [
        pltpu.VMEM((1, 1, M), BF16),
        pltpu.VMEM((M,), BF16),
        pltpu.VMEM((M, HD), BF16),
        pltpu.VMEM((M * H, D), BF16),
        pltpu.VMEM((C * H, D), BF16),
        pltpu.VMEM((S, C), BF16),
        pltpu.VMEM((C * H, D), BF16),
        pltpu.VMEM((HD, M), BF16),
        pltpu.VMEM((H, S, D), BF16),
        pltpu.VMEM((H, S, D), BF16),
    ] + [pltpu.VMEM((n, M), BF16) for n in WO_SIZES] + [
        pltpu.VMEM((HD, 128), BF16),
        pltpu.VMEM((H, R, D), BF16),
        pltpu.VMEM((H, R, S), BF16),
        pltpu.VMEM((H, R, D), F32),
        pltpu.VMEM((H, R, D), F32),
        pltpu.VMEM(((H - VH0) * D, D), F32),
        pltpu.VMEM((1, 1, M), BF16),
    ]
    return pl.pallas_call(
        _kernel,
        out_shape=jax.ShapeDtypeStruct((1, 1, M), BF16),
        in_specs=[any_spec] * len(args),
        out_specs=any_spec,
        scratch_shapes=scratch,
        compiler_params=pltpu.CompilerParams(vmem_limit_bytes=120 * 1024 * 1024),
    )(*args)
```
